```python
import os as _os
_os.environ.setdefault("JAX_PLATFORMS", "cpu")
import jax
import jax.numpy as jnp

def _softmax(x, axis=-1):
    return jax.nn.softmax(x, axis=axis)
def _gelu(x):
    return jax.nn.gelu(x, approximate=True)
def _silu(x):
    return jax.nn.silu(x)
def _sigmoid(x):
    return jax.nn.sigmoid(x)
def _layernorm(x, axis=-1, eps=1e-5):
    m = jnp.mean(x, axis=axis, keepdims=True)
    v = jnp.var(x, axis=axis, keepdims=True)
    return (x - m) / jnp.sqrt(v + eps)
def _scatter_add(tgt, idx, src, axis=0):
    return tgt.at[idx].add(src)
def _segment_sum(src, seg, n):
    return jax.ops.segment_sum(src, seg, n)
class _Rng:
    def __init__(self, key):
        self._k = key
    def _next(self):
        self._k, sub = jax.random.split(self._k)
        return sub
    def normal(self, shape):
        return jax.random.normal(self._next(), shape, dtype=jnp.bfloat16)
    def randint(self, lo, hi, shape):
        return jax.random.randint(self._next(), shape, lo, hi, dtype=jnp.int32)
    def uniform(self, shape, lo=0.0, hi=1.0):
        return jax.random.uniform(self._next(), shape, jnp.bfloat16, lo, hi)
    def permutation(self, n):
        return jax.random.permutation(self._next(), n)


kernel_name = 'sequential_preLN__softmax_full_mha__dense_activation_gelu__prompt'

def setup_inputs():
    _rng = _Rng(jax.random.key(int.from_bytes(__import__("os").urandom(4), "little")))
    _w = (lambda a: (lambda t: t.astype(jnp.bfloat16) if jnp.issubdtype(t.dtype, jnp.floating) else t)(jnp.asarray(a)))
    def _A_setup():
        B, S, D = 1, 2048, 640
        return {
            "x": _w((lambda *s: _rng.normal(s) * 0.05)(B, S, D)),
            "wqkv": _w((lambda *s: _rng.normal(s) * 0.05)(D, 3 * D)),
            "wo": _w((lambda *s: _rng.normal(s) * 0.05)(D, D)),
        }
    _A_in = _A_setup()

    def _B_setup():
        B, S, D, F = 1, 2048, 640, 1536
        return {
            "x": _w((lambda *s: _rng.normal(s) * 0.05)(B, S, D)),
            "w1": _w((lambda *s: _rng.normal(s) * 0.4)(D, F) * (D ** -0.5)),
            "b1": _w((lambda *s: _rng.normal(s) * 0.4)(F) * 0.01),
            "w2": _w((lambda *s: _rng.normal(s) * 0.4)(F, D) * (F ** -0.5)),
            "b2": _w((lambda *s: _rng.normal(s) * 0.05)(D) * 0.01),
        }
    _B_in = _B_setup()

    return {
        "A_x": _A_in["x"],
        "A_wqkv": _A_in["wqkv"],
        "A_wo": _A_in["wo"],
        "B_x": _B_in["x"],
        "B_w1": _B_in["w1"],
        "B_b1": _B_in["b1"],
        "B_w2": _B_in["w2"],
        "B_b2": _B_in["b2"],
    }

def reference(A_x, A_wqkv, A_wo, B_x, B_w1, B_b1, B_w2, B_b2):
    def _A_ref(x, wqkv, wo):
        B, S, D = x.shape
        H = 32; Dh = D // H
        qkv = (lambda x, *d: x.transpose(*d))((x @ wqkv).reshape(B, S, 3, H, Dh), 2, 0, 3, 1, 4)
        q, k, v = qkv[0], qkv[1], qkv[2]
        scale = Dh ** -0.5
        scores = jnp.einsum("bhqd,bhkd->bhqk", q, k) * scale
        p = _softmax(scores, axis=-1)
        o = jnp.einsum("bhqk,bhkd->bhqd", p, v)
        return (lambda x, *d: x.transpose(*d))(o, 0, 2, 1, 3).reshape(B, S, D) @ wo

    def _B_ref(x, w1, b1, w2, b2):
        h = jnp.einsum("bsd,df->bsf", x, w1) + b1
        h = _gelu(h)
        return jnp.einsum("bsf,fd->bsd", h, w2) + b2

    x = A_x
    h = x + _A_ref(_layernorm(x, axis=-1), A_wqkv, A_wo)
    h2 = h + _B_ref(_layernorm(h, axis=-1), B_w1, B_b1, B_w2, B_b2)
    return h2
```

```python
import functools, math
import jax, jax.numpy as jnp
from jax import lax
from jax.experimental import pallas as pl
from jax.experimental.pallas import tpu as pltpu

S, D, H, DH, F = 2048, 640, 32, 20, 1536
EPS = 1e-5
QSCALE = (DH ** -0.5) * math.log2(math.e)
NT = (((1,), (1,)), ((), ()))
f32, bf16 = jnp.float32, jnp.bfloat16

def _ln(x):
    m = jnp.mean(x, axis=-1, keepdims=True)
    xc = x - m
    v = jnp.mean(xc * xc, axis=-1, keepdims=True)
    return xc * lax.rsqrt(v + EPS)

def make_kernel(TQ=512, RC=256, FC=256, SK=1, QC=512, DH2=256, QB=128, SUB=128):
    TK = 512 * 128 // QB
    NC = S // TK
    NQ = S // TQ
    NR = S // RC
    NB = TQ // QB
    NSB = 4
    def kernel(x_hbm, wqkv_hbm, wo_hbm, w1_hbm, b1_ref, w2_hbm, b2_ref, o_ref,
               x_ref, wqkv_ref, wo_ref, w1_ref, w2_ref, xn_ref,
               kg_ref, qw_ref, vtp_ref, wqvt_ref, m_ref, acc_ref, ot_ref, z_ref, xsem, wsem, *s_refs):
        step = pl.program_id(0)
        z_ref[0] = jnp.minimum(step, 0)

        def xcopy(r):
            r0 = r * RC if isinstance(r, int) else pl.multiple_of(r * RC, RC)
            return pltpu.make_async_copy(x_hbm.at[pl.ds(r0, RC), :], x_ref.at[pl.ds(r0, RC), :], xsem.at[r])
        def wcopy(i):
            if i < 3:
                return pltpu.make_async_copy(wqkv_hbm.at[:, pl.ds(i * D, D)], wqkv_ref.at[i], wsem.at[i])
            src, dst = [(wo_hbm, wo_ref), (w1_hbm, w1_ref), (w2_hbm, w2_ref)][i - 3]
            return pltpu.make_async_copy(src, dst, wsem.at[i])

        def qprep(h, q0):
            start = h * DH
            g0 = start // 128
            lo = start - g0 * 128
            gi = g0 + 5 if lo + DH > 128 else g0
            a = (lo // 16) * 16
            w = qw_ref[h, :, pl.ds(q0, QB)]
            if a + 32 <= 128:
                parts = []
                if a > 0:
                    parts.append(jnp.zeros((a, QB), bf16))
                parts.append(w)
                if a + 32 < 128:
                    parts.append(jnp.zeros((128 - a - 32, QB), bf16))
            else:
                parts = [w[16:32], jnp.zeros((96, QB), bf16), w[0:16]]
            return gi, jnp.concatenate(parts, axis=0)

        def smpv(h, s_ref, m, c, acc, zz):
            sl = slice(c * TK, (c + 1) * TK)
            p = jnp.exp2(s_ref[zz, sl, :] - m).astype(bf16)
            o = jnp.dot(vtp_ref[h, :, sl], p, preferred_element_type=f32)
            return o if acc is None else acc + o

        def finalize(h, a, lq):
            r0 = (h // 2) * 40
            if h % 2 == 0:
                a = a * (1.0 / a[23:24])
                ot_ref[r0:r0 + 20, pl.ds(lq, QB)] = a[0:20]
            else:
                a = a * (1.0 / a[0:1])
                ot_ref[r0 + 20:r0 + 40, pl.ds(lq, QB)] = a[4:24]

        def stage(hq, q0, sq_ref, cur, prev):
            gi, qtm = qprep(hq, q0)
            zz = z_ref[0]
            m8 = None
            acc = None
            for c in range(NC):
                for u in range(TK // SUB):
                    sl = slice(c * TK + u * SUB, c * TK + (u + 1) * SUB)
                    s = jnp.dot(kg_ref[gi, sl, :], qtm, preferred_element_type=f32)
                    sq_ref[0, sl, :] = s
                    cm = jnp.max(s.reshape(SUB // 8, 8, QB), axis=0)
                    m8 = cm if m8 is None else jnp.maximum(m8, cm)
                if c < SK:
                    if prev is not None:
                        hpp, spp, mpp, app, lq = prev
                        app = smpv(hpp, spp, mpp, NC - SK + c, app, zz)
                        prev = (hpp, spp, mpp, app, lq)
                        if c == SK - 1:
                            finalize(hpp, app, lq)
                elif cur is not None:
                    acc = smpv(cur[0], cur[1], cur[2], c - SK, acc, zz)
            return jnp.max(m8, axis=0, keepdims=True), acc

        @pl.when(step == 0)
        def _prologue():
            xcopy(0).start()
            wcopy(1).start()
            xcopy(1).start()
            xcopy(2).start()

            def ln_chunk(r):
                r0 = r * RC if isinstance(r, int) else pl.multiple_of(r * RC, RC)
                xn_ref[pl.ds(r0, RC), :] = _ln(x_ref[pl.ds(r0, RC), :].astype(f32)).astype(bf16)
            lane = lax.broadcasted_iota(jnp.int32, (RC, 128), 1)
            def k_chunk(r):
                r0 = r * RC if isinstance(r, int) else pl.multiple_of(r * RC, RC)
                k = jnp.dot(xn_ref[pl.ds(r0, RC), :], wqkv_ref[1], preferred_element_type=f32).astype(bf16)
                for g in range(5):
                    kg_ref[g, pl.ds(r0, RC), :] = k[:, 128 * g:128 * (g + 1)]
                for j in range(4):
                    kg_ref[5 + j, pl.ds(r0, RC), :] = jnp.where(lane >= 64, k[:, 128 * j:128 * (j + 1)], k[:, 128 * (j + 1):128 * (j + 2)])

            row24 = lax.broadcasted_iota(jnp.int32, (24, QC), 0)
            row32 = lax.broadcasted_iota(jnp.int32, (32, QC), 0)
            def qv_chunk(r):
                r0 = r * QC if isinstance(r, int) else pl.multiple_of(r * QC, QC)
                qvt = lax.dot_general(wqvt_ref[...].reshape(2 * D, D), xn_ref[pl.ds(r0, QC), :], NT, preferred_element_type=f32)
                qt = qvt[0:D] * QSCALE
                for h in range(H):
                    w0 = (h * DH // 16) * 16
                    off = h * DH - w0
                    qw_ref[h, :, pl.ds(r0, QC)] = jnp.where((row32 >= off) & (row32 < off + DH), qt[w0:w0 + 32], 0.0).astype(bf16)
                vt = qvt[D:2 * D]
                for h in range(H):
                    i = h % 2
                    w0 = 40 * (h // 2) + 16 * i
                    onerow = 0 if i == 1 else 23
                    vtp_ref[h, :, pl.ds(r0, QC)] = jnp.where(row24 == onerow, 1.0, vt[w0:w0 + 24])

            s_refs[NSB - 1][0, (NC - SK) * TK:, :] = jnp.zeros((SK * TK, QB), f32)
            m_ref[1:2, :] = jnp.zeros((1, QB), f32)
            acc_ref[...] = jnp.ones((24, QB), f32)

            xcopy(0).wait()
            xcopy(3).start()
            xcopy(4).start()
            xcopy(5).start()
            wcopy(0).start()
            ln_chunk(0)
            xcopy(1).wait()
            xcopy(2).wait()
            wcopy(1).wait()
            xcopy(6).start()
            xcopy(7).start()
            wcopy(2).start()
            k_chunk(0)
            ln_chunk(1)
            k_chunk(1)
            ln_chunk(2)

            def kbody(i, carry):
                r = 2 + 3 * i
                xcopy(r + 1).wait()
                xcopy(r + 2).wait()
                @pl.when(i == 0)
                def _():
                    xcopy(5).wait()
                pltpu.make_async_copy(wqkv_hbm.at[:, pl.ds(0, D)], wqkv_ref.at[2 * i], wsem.at[2 * i]).wait()
                k_chunk(r)
                ln_chunk(r + 1)
                k_chunk(r + 1)
                wqvt_ref[i] = wqkv_ref[2 * i].T
                ln_chunk(r + 2)
                k_chunk(r + 2)
                ln_chunk(jnp.minimum(r + 3, NR - 1))
                return carry
            lax.fori_loop(0, 2, kbody, 0)
            for i in range(3, 6):
                wcopy(i).start()

            def qvbody(r, carry):
                qv_chunk(r)
                return carry
            lax.fori_loop(0, S // QC, qvbody, 0)
            m_ref[0:1, :] = stage(0, 0, s_refs[0], None, None)[0]
            for i in range(3, 6):
                wcopy(i).wait()

        q0 = pl.multiple_of(step * TQ, TQ)

        def bbody(b, carry):
            lq = pl.multiple_of(b * QB, QB)
            lqp = pl.multiple_of(jnp.where(b == 0, NB - 1, b - 1) * QB, QB)
            gq = pl.multiple_of(q0 + lq, QB)
            gqn = pl.multiple_of(jnp.minimum(gq + QB, S - QB), QB)
            mp = m_ref[0:1, :]
            mpp = m_ref[1:2, :]
            app = acc_ref[...]
            for hp in range(H):
                hq, qq = (hp + 1, gq) if hp + 1 < H else (0, gqn)
                hpp = (hp - 1) % H
                mq, ap = stage(hq, qq, s_refs[(hp + 1) % NSB],
                               (hp, s_refs[hp % NSB], mp),
                               (hpp, s_refs[hpp % NSB], mpp, app, lq if hp > 0 else lqp))
                mpp, app, mp = mp, ap, mq
            m_ref[0:1, :] = mp
            m_ref[1:2, :] = mpp
            acc_ref[...] = app
            return carry
        lax.fori_loop(0, NB, bbody, 0)

        zz = z_ref[0]
        app = acc_ref[...]
        mpp = m_ref[1:2, :]
        for c in range(NC - SK, NC):
            app = smpv(H - 1, s_refs[(H - 1) % NSB], mpp, c, app, zz)
        finalize(H - 1, app, (NB - 1) * QB)

        NH = TQ // DH2
        hres, hn, acc = [None] * NH, [None] * NH, [None] * NH
        b2 = b2_ref[...].astype(f32)
        for a in range(NH):
            o = ot_ref[:, a * DH2:(a + 1) * DH2].T.astype(bf16)
            hres[a] = x_ref[pl.ds(q0 + a * DH2, DH2), :].astype(f32) + jnp.dot(o, wo_ref[...], preferred_element_type=f32)
        for a in range(NH):
            hn[a] = _ln(hres[a]).astype(bf16)
            acc[a] = hres[a] + b2
        for c in range(F // FC):
            us = []
            for a in range(NH):
                u = jnp.dot(hn[a], w1_ref[:, c * FC:(c + 1) * FC], preferred_element_type=f32) + b1_ref[:, c * FC:(c + 1) * FC].astype(f32)
                us.append(jax.nn.gelu(u, approximate=True).astype(bf16))
            for a in range(NH):
                acc[a] = acc[a] + jnp.dot(us[a], w2_ref[c * FC:(c + 1) * FC, :], preferred_element_type=f32)
        for a in range(NH):
            o_ref[a * DH2:(a + 1) * DH2, :] = acc[a].astype(o_ref.dtype)

    def fn(A_x, A_wqkv, A_wo, B_x, B_w1, B_b1, B_w2, B_b2):
        x = A_x.reshape(S, D)
        full = lambda shape: pl.BlockSpec(shape, lambda i: (0,) * len(shape))
        anyspec = pl.BlockSpec(memory_space=pl.ANY)
        out = pl.pallas_call(
            kernel,
            grid=(NQ,),
            in_specs=[anyspec, anyspec, anyspec, anyspec, full((1, F)), anyspec, full((1, D))],
            out_specs=pl.BlockSpec((TQ, D), lambda i: (i, 0)),
            out_shape=jax.ShapeDtypeStruct((S, D), bf16),
            scratch_shapes=[
                pltpu.VMEM((S, D), bf16),
                pltpu.VMEM((3, D, D), bf16),
                pltpu.VMEM((D, D), bf16),
                pltpu.VMEM((D, F), bf16),
                pltpu.VMEM((F, D), bf16),
                pltpu.VMEM((S, D), bf16),
                pltpu.VMEM((9, S, 128), bf16),
                pltpu.VMEM((H, 32, S), bf16),
                pltpu.VMEM((H, 24, S), f32),
                pltpu.VMEM((2, D, D), bf16),
                pltpu.VMEM((8, QB), f32),
                pltpu.VMEM((24, QB), f32),
                pltpu.VMEM((D, TQ), f32),
                pltpu.SMEM((1,), jnp.int32),
                pltpu.SemaphoreType.DMA((NR,)),
                pltpu.SemaphoreType.DMA((6,)),
            ] + [pltpu.VMEM((1, S, QB), f32) for _ in range(NSB)],
            compiler_params=pltpu.CompilerParams(dimension_semantics=("arbitrary",), vmem_limit_bytes=110 * 1024 * 1024),
        )(x, A_wqkv, A_wo, B_w1, B_b1.reshape(1, F), B_w2, B_b2.reshape(1, D))
        return out.reshape(1, S, D)
    return fn


_FN = make_kernel(SK=2)


@jax.jit
def pallas_sequential_preLN__softmax_full_mha__dense_activation_gelu__prompt_kernel(
    A_x: jax.Array,
    A_wqkv: jax.Array,
    A_wo: jax.Array,
    B_x: jax.Array,
    B_w1: jax.Array,
    B_b1: jax.Array,
    B_w2: jax.Array,
    B_b2: jax.Array,
):
    return _FN(A_x, A_wqkv, A_wo, B_x, B_w1, B_b1, B_w2, B_b2)
```

```python
import functools, math
import jax, jax.numpy as jnp
from jax import lax
from jax.experimental import pallas as pl
from jax.experimental.pallas import tpu as pltpu

S, D, H, DH, F = 2048, 640, 32, 20, 1536
EPS = 1e-5
QSCALE = (DH ** -0.5) * math.log2(math.e)
NT = (((1,), (1,)), ((), ()))
f32, bf16, u32 = jnp.float32, jnp.bfloat16, jnp.uint32

TSAFE = 60.0
VSC = TSAFE * 2.0 ** -50

def _ln(x):
    m = jnp.mean(x, axis=-1, keepdims=True)
    xc = x - m
    v = jnp.mean(xc * xc, axis=-1, keepdims=True)
    return xc * lax.rsqrt(v + EPS)

def make_kernel(TQ=512, RC=256, FC=256, SK=1, QC=512, DH2=128, QB=128, OFF=224, NCH=4, THIN=1, KPH=2, NSB=4, PB=1, ORD=2, PRE=0):
    TK = 512
    NC = S // TK
    NQ = S // TQ
    NR = S // RC
    NB = TQ // QB
    NG16 = OFF // 16
    order = [[0, 2, 1, 3], [1, 2, 3, 0], [0, 2, 3, 1], [0, 1, 3, 2]][ORD]
    RANGES2 = []
    for var in range(4):
        short = []
        for c_ in order:
            us = [[0, 1, 2, 3], [2, 3, 0, 1], [1, 2, 3, 0], [3, 0, 1, 2]][var] if NG16 % 2 else [[0, 1, 2, 3], [2, 3, 0, 1]][var % 2]
            short += [c_ * 4 + u_ for u_ in us]
        short = set(short[:NG16])
        rg, pos = [], OFF
        for t_ in range(16):
            n_ = 112 if t_ in short else 128
            rg.append((pos, pos + n_))
            pos += n_
        assert pos == S
        RANGES2.append(rg)
    NP = OFF // 8
    PSTART = [(c_ * NP) // 4 for c_ in range(5)]

    def kernel(x_hbm, wqkv_hbm, wo_hbm, w1_hbm, b1_hbm, w2_hbm, b2_hbm, o_hbm,
               x_ref, wqkv_ref, wo_ref, w1_ref, w2_ref, xn_ref,
               kg_ref, qw_ref, vtp_ref, wqvt_ref, m_ref, acc_ref, ot_ref, kb_ref, z_ref, ok_ref, xsem, wsem, osem, *rest):
        s_refs, (fl_ref, wq_ref, b1_ref, b2_ref) = list(zip(rest[:NSB], rest[NSB:2 * NSB])), rest[2 * NSB:]
        step = pl.program_id(0)
        z_ref[0] = jnp.minimum(step, 0)
        ob_ref = xn_ref

        def xcopy(r):
            return pltpu.make_async_copy(x_hbm.at[pl.ds(r * RC, RC), :], x_ref.at[pl.ds(r * RC, RC), :], xsem.at[r])
        def wcopy(i):
            if i < 3:
                return pltpu.make_async_copy(wqkv_hbm.at[:, pl.ds(i * D, D)], wqkv_ref.at[i], wsem.at[i])
            src, dst = [(wo_hbm, wo_ref), (w1_hbm, w1_ref), (w2_hbm, w2_ref), (b1_hbm, b1_ref), (b2_hbm, b2_ref)][i - 3]
            return pltpu.make_async_copy(src, dst, wsem.at[i])
        def ocopy(i):
            r0 = i * DH2 if isinstance(i, int) else pl.multiple_of(i * DH2, DH2)
            return pltpu.make_async_copy(ob_ref.at[pl.ds(r0, DH2), :], o_hbm.at[pl.ds(r0, DH2), :], osem.at[i])

        def qprep(h, q0):
            start = h * DH
            g0 = start // 128
            lo = start - g0 * 128
            gi = g0 + 5 if lo + DH > 128 else g0
            a = (lo // 16) * 16
            w = pltpu.bitcast(qw_ref[h, :, pl.ds(q0, QB)], bf16)
            if a + 32 <= 128:
                parts = []
                if a > 0:
                    parts.append(jnp.zeros((a, QB), bf16))
                parts.append(w)
                if a + 32 < 128:
                    parts.append(jnp.zeros((128 - a - 32, QB), bf16))
            else:
                parts = [w[16:32], jnp.zeros((96, QB), bf16), w[0:16]]
            wf = w.astype(f32)
            off = start - (start // 16) * 16
            qrows = [jnp.broadcast_to(wf[off + d:off + d + 1], (8, QB)) for d in range(DH)]
            return gi, jnp.concatenate(parts, axis=0), qrows

        def smpv(h, s_ref, m, c, acc, zz):
            s_ref, so_ref = s_ref
            sl = slice(c * TK, (c + 1) * TK)
            if c == 0:
                tail = s_ref[zz, TK - 8:TK, :]
                tail = jnp.maximum(tail, jnp.minimum(m, tail))
                sv = jnp.concatenate([so_ref[zz], s_ref[zz, OFF:TK - 8, :], tail], axis=0)
            else:
                sv = s_ref[zz, sl, :]
            p = jnp.exp2(sv)
            if PB:
                p = p.astype(bf16)
            o = jnp.dot(vtp_ref[h, :, sl], p, preferred_element_type=f32)
            return o if acc is None else acc + o

        def finalize(pair, odd, a, lq, ok=None):
            if not odd:
                a = (a * (1.0 / a[23:24]))[0:20]
                rows = slice(0, 20)
            else:
                a = (a * (1.0 / a[0:1]))[4:24]
                rows = slice(20, 40)
            if ok is not None:
                a = jnp.where(ok, a, ot_ref[pair, rows, pl.ds(lq, QB)])
            ot_ref[pair, rows, pl.ds(lq, QB)] = a

        def stage(hq, q0, sq_ref, cur, prev):
            sq_ref, so_ref = sq_ref
            gi, qtm, qrows = qprep(hq, q0)
            zz = z_ref[0]
            m8 = None
            acc = None
            def vpu_piece(g):
                parts = []
                for ch in range(NCH):
                    sv = None
                    for d in range(ch, DH, NCH):
                        tt = kb_ref[g, (hq * DH + d) * 8:(hq * DH + d + 1) * 8, :] * qrows[d]
                        sv = tt if sv is None else sv + tt
                    parts.append(sv)
                while len(parts) > 1:
                    parts = [parts[i] + parts[i + 1] if i + 1 < len(parts) else parts[i] for i in range(0, len(parts), 2)]
                so_ref[0, g * 8:(g + 1) * 8, :] = parts[0]
                return parts[0]
            for c in range(NC):
                ss = []
                for u in range(4):
                    lo_, hi_ = RANGES2[hq % 4][c * 4 + u]
                    s = jnp.dot(pltpu.bitcast(kg_ref[gi, lo_ // 2:hi_ // 2, :], bf16), qtm, preferred_element_type=f32)
                    sq_ref[0, lo_:hi_, :] = s
                    ss.append(s.reshape((hi_ - lo_) // 8, 8, QB))
                PPC = PSTART[c + 1] - PSTART[c]
                for qd in range(PPC):
                    cm = jnp.max(jnp.concatenate([ss[u][(qd * ss[u].shape[0]) // PPC:((qd + 1) * ss[u].shape[0]) // PPC] for u in range(0, 4, THIN)], axis=0), axis=0)
                    if PRE:
                        v = vpu_piece(PSTART[c] + qd)
                        m8 = v if m8 is None else jnp.maximum(m8, v)
                        m8 = jnp.maximum(m8, cm)
                    else:
                        m8 = cm if m8 is None else jnp.maximum(m8, cm)
                        m8 = jnp.maximum(m8, vpu_piece(PSTART[c] + qd))
                if c < SK:
                    if prev is not None:
                        hpp, spp, mpp, app, lq = prev
                        app = smpv(hpp, spp, mpp, NC - SK + c, app, zz)
                        prev = (hpp, spp, mpp, app, lq)
                        if c == SK - 1:
                            finalize(hpp // 2, hpp % 2 == 1, app, lq)
                elif cur is not None:
                    acc = smpv(cur[0], cur[1], cur[2], c - SK, acc, zz)
            return jnp.max(m8, axis=0, keepdims=True), acc

        @pl.when(step == 0)
        def _prologue():
            xcopy(0).start()
            wcopy(1).start()
            xcopy(1).start()
            for r in range(2, 5):
                xcopy(r).start(priority=1)

            def ln_chunk(r):
                r0 = r * RC
                xn_ref[pl.ds(r0, RC), :] = _ln(x_ref[pl.ds(r0, RC), :].astype(f32)).astype(bf16)
            lane = lax.broadcasted_iota(jnp.int32, (RC // 2, 128), 1)
            def k_chunk(r):
                r0 = r * RC
                k = jnp.dot(xn_ref[pl.ds(r0, RC), :], wqkv_ref[1], preferred_element_type=f32).astype(bf16)
                k = pltpu.bitcast(k, u32)
                for g in range(5):
                    kg_ref[g, pl.ds(r0 // 2, RC // 2), :] = k[:, 128 * g:128 * (g + 1)]
                for j in range(4):
                    kg_ref[5 + j, pl.ds(r0 // 2, RC // 2), :] = jnp.where(lane >= 64, k[:, 128 * j:128 * (j + 1)], k[:, 128 * (j + 1):128 * (j + 2)])

            def bcast(i0, n, cols):
                hb = i0 * 8 if isinstance(i0, int) else pl.multiple_of(i0 * 8, 8)
                kks = {}
                for col in cols:
                    g = col // 128
                    if g not in kks:
                        kks[g] = kg_ref[g, pl.ds(hb, n * 8), :]
                    cc = col - g * 128
                    bb = jnp.broadcast_to(kks[g][:, cc:cc + 1], (n * 8, 128))
                    bbf = pltpu.bitcast(bb, bf16).astype(f32)
                    for gg in range(2 * n):
                        kb_ref[2 * i0 + gg, col * 8:(col + 1) * 8, :] = bbf[gg * 8:(gg + 1) * 8]

            row24 = lax.broadcasted_iota(jnp.int32, (24, QC), 0)
            row32 = lax.broadcasted_iota(jnp.int32, (32, QC), 0)
            NQV = S // QC
            PERQ = (NG16 - KPH) // NQV
            assert PERQ * NQV + KPH == NG16
            def qv_chunk(r):
                r0 = pl.multiple_of(r * QC, QC)
                qvt = lax.dot_general(wqvt_ref[...].reshape(2 * D, D), xn_ref[pl.ds(r0, QC), :], NT, preferred_element_type=f32)
                qt = qvt[0:D] * QSCALE
                bcast(KPH + r * PERQ, PERQ, range(D))
                for h in range(H):
                    w0 = (h * DH // 16) * 16
                    off = h * DH - w0
                    w = jnp.where((row32 >= off) & (row32 < off + DH), qt[w0:w0 + 32], 0.0).astype(bf16)
                    qw_ref[h, :, pl.ds(r0, QC)] = pltpu.bitcast(w, u32)
                vt = qvt[D:2 * D]
                va = jnp.max(jnp.abs(vt).reshape(D // 8, 8, QC), axis=0)
                va = jnp.max(va.reshape(8, QC // 128, 128).transpose(1, 0, 2), axis=0) if False else functools.reduce(jnp.maximum, [va[:, i * 128:(i + 1) * 128] for i in range(QC // 128)])
                fl_ref[8:16, :] = jnp.maximum(fl_ref[8:16, :], va * VSC)
                for h in range(H):
                    i = h % 2
                    w0 = 40 * (h // 2) + 16 * i
                    onerow = 0 if i == 1 else 23
                    vtp_ref[h, :, pl.ds(r0, QC)] = jnp.where(row24 == onerow, 1.0, vt[w0:w0 + 24])

            s_refs[NSB - 1][0][0, (NC - SK) * TK:, :] = jnp.zeros((SK * TK, QB), f32)
            m_ref[1:2, :] = jnp.zeros((1, QB), f32)
            acc_ref[...] = jnp.ones((24, QB), f32)
            fl_ref[8:16, :] = jnp.zeros((8, QB), f32)

            def kb_part(j):
                if KPH:
                    lo_, hi_ = (j * D) // 7, ((j + 1) * D) // 7
                    bcast(0, KPH, range(lo_, hi_))

            xcopy(0).wait()
            for r in range(5, 8):
                xcopy(r).start(priority=1)
            ln_chunk(0)
            xcopy(1).wait()
            wcopy(1).wait()
            wcopy(0).start(priority=1)
            wcopy(2).start(priority=1)
            k_chunk(0)
            ln_chunk(1)
            for r in range(2, 5):
                xcopy(r).wait()
            for i in range(3, 8):
                wcopy(i).start(priority=1)
            for r in range(1, 4):
                k_chunk(r)
                kb_part(r - 1)
                ln_chunk(r + 1)
            for r in range(5, 8):
                xcopy(r).wait()
            wcopy(0).wait()
            wcopy(2).wait()
            for r in range(4, 8):
                k_chunk(r)
                kb_part(r - 1)
                if r + 1 < NR:
                    ln_chunk(r + 1)
            wqvt_ref[0] = wqkv_ref[0].T
            wqvt_ref[1] = wqkv_ref[2].T

            def qvbody(r, carry):
                qv_chunk(r)
                return carry
            lax.fori_loop(0, S // QC, qvbody, 0)
            m_ref[0:1, :] = stage(0, 0, s_refs[0], None, None)[0]
            for i in range(3, 8):
                wcopy(i).wait()

        q0 = pl.multiple_of(step * TQ, TQ)
        fl_ref[0:8, :] = fl_ref[8:16, :]

        def bbody(b, carry):
            lq = pl.multiple_of(b * QB, QB)
            lqp = pl.multiple_of(jnp.where(b == 0, NB - 1, b - 1) * QB, QB)
            gq = pl.multiple_of(q0 + lq, QB)
            gqn = pl.multiple_of(jnp.minimum(gq + QB, S - QB), QB)
            mp = m_ref[0:1, :]
            mpp = m_ref[1:2, :]
            app = acc_ref[...]
            fl = fl_ref[0:8, :]
            for hp in range(H):
                fl = jnp.maximum(fl, jnp.abs(mp))
                if hp == H - 1:
                    fl_ref[0:8, :] = fl
                    ok_ref[0] = jnp.where(jnp.max(fl) <= TSAFE, 1, 0).astype(jnp.int32)
                hq, qq = (hp + 1, gq) if hp + 1 < H else (0, gqn)
                hpp = (hp - 1) % H
                mq, ap = stage(hq, qq, s_refs[(hp + 1) % NSB],
                               (hp, s_refs[hp % NSB], mp),
                               (hpp, s_refs[hpp % NSB], mpp, app, lq if hp > 0 else lqp))
                mpp, app, mp = mp, ap, mq
            m_ref[0:1, :] = mp
            m_ref[1:2, :] = mpp
            acc_ref[...] = app
            return carry
        lax.fori_loop(0, NB, bbody, 0)

        ok = ok_ref[0] == 1

        @pl.when(jnp.logical_not(ok))
        def _slow_path():
            sw_ref = s_refs[1][0]
            def one(h, pair, odd, lq, gq):
                start = h * DH
                g0 = start // 128
                lo = start - g0 * 128
                gi = jnp.where(lo + DH > 128, g0 + 5, g0)
                a0 = pl.multiple_of((lo // 16) * 8, 8)
                a1 = pl.multiple_of((a0 + 8) % 64, 8)
                w = qw_ref[h, :, pl.ds(gq, QB)]
                wq_ref[...] = jnp.zeros((64, QB), u32)
                wq_ref[pl.ds(a0, 8), :] = w[0:8]
                wq_ref[pl.ds(a1, 8), :] = w[8:16]
                qtm = pltpu.bitcast(wq_ref[...], bf16)
                def p1(c, m8):
                    r0 = pl.multiple_of(c * 128, 128)
                    s = jnp.dot(pltpu.bitcast(kg_ref[gi, pl.ds(pl.multiple_of(c * 64, 64), 64), :], bf16), qtm, preferred_element_type=f32)
                    sw_ref[0, pl.ds(r0, 128), :] = s
                    return jnp.maximum(m8, jnp.max(s.reshape(16, 8, QB), axis=0))
                m8 = lax.fori_loop(0, S // 128, p1, jnp.full((8, QB), -jnp.inf, f32))
                m = jnp.max(m8, axis=0, keepdims=True)
                def p2(c, acc):
                    r0 = pl.multiple_of(c * 128, 128)
                    p = jnp.exp2(sw_ref[0, pl.ds(r0, 128), :] - m).astype(bf16)
                    return acc + jnp.dot(vtp_ref[h, :, pl.ds(r0, 128)], p, preferred_element_type=f32)
                acc = lax.fori_loop(0, S // 128, p2, jnp.zeros((24, QB), f32))
                finalize(pair, odd, acc, lq)
            def sbody(i, carry):
                b = i // (H // 2)
                pair = i - b * (H // 2)
                lq = pl.multiple_of(b * QB, QB)
                gq = pl.multiple_of(q0 + lq, QB)
                one(2 * pair, pair, False, lq, gq)
                one(2 * pair + 1, pair, True, lq, gq)
                return carry
            lax.fori_loop(0, NB * (H // 2), sbody, 0)

        zz = z_ref[0]
        app = acc_ref[...]
        mpp = m_ref[1:2, :]
        for c in range(NC - SK, NC):
            app = smpv(H - 1, s_refs[(H - 1) % NSB], mpp, c, app, zz)
        finalize((H - 1) // 2, True, app, (NB - 1) * QB, ok)

        NH = TQ // DH2
        NF = F // FC
        hres, hn = [None] * NH, [None] * NH
        b2 = b2_ref[...].astype(f32)[None, :]
        for a in range(NH):
            o = ot_ref[:, :, a * DH2:(a + 1) * DH2].reshape(D, DH2).T.astype(bf16)
            hres[a] = x_ref[pl.ds(q0 + a * DH2, DH2), :].astype(f32) + jnp.dot(o, wo_ref[...], preferred_element_type=f32)
        def up(a, c):
            if c == 0:
                hn[a] = _ln(hres[a]).astype(bf16)
            u = jnp.dot(hn[a], w1_ref[:, c * FC:(c + 1) * FC], preferred_element_type=f32) + b1_ref[c * FC:(c + 1) * FC].astype(f32)[None, :]
            return jax.nn.gelu(u, approximate=True).astype(bf16)
        seq = [(a, c) for a in range(NH) for c in range(NF)]
        g = up(*seq[0])
        acc = None
        for i, (a, c) in enumerate(seq):
            gn = up(*seq[i + 1]) if i + 1 < len(seq) else None
            if c == 0:
                acc = hres[a] + b2
            acc = acc + jnp.dot(g, w2_ref[c * FC:(c + 1) * FC, :], preferred_element_type=f32)
            if c == NF - 1:
                ob_ref[pl.ds(q0 + a * DH2, DH2), :] = acc.astype(bf16)
                ocopy(step * NH + a).start()
            g = gn

        @pl.when(step == NQ - 1)
        def _():
            for i in range(S // DH2):
                ocopy(i).wait()

    def fn(A_x, A_wqkv, A_wo, B_x, B_w1, B_b1, B_w2, B_b2):
        x = A_x.reshape(S, D)
        anyspec = pl.BlockSpec(memory_space=pl.ANY)
        out = pl.pallas_call(
            kernel,
            grid=(NQ,),
            in_specs=[anyspec] * 7,
            out_specs=anyspec,
            out_shape=jax.ShapeDtypeStruct((S, D), bf16),
            scratch_shapes=[
                pltpu.VMEM((S, D), bf16),
                pltpu.VMEM((3, D, D), bf16),
                pltpu.VMEM((D, D), bf16),
                pltpu.VMEM((D, F), bf16),
                pltpu.VMEM((F, D), bf16),
                pltpu.VMEM((S, D), bf16),
                pltpu.VMEM((9, S // 2, 128), u32),
                pltpu.VMEM((H, 16, S), u32),
                pltpu.VMEM((H, 24, S), f32),
                pltpu.VMEM((2, D, D), bf16),
                pltpu.VMEM((8, QB), f32),
                pltpu.VMEM((24, QB), f32),
                pltpu.VMEM((H // 2, 40, TQ), f32),
                pltpu.VMEM((OFF // 8, D * 8, 128), f32),
                pltpu.SMEM((1,), jnp.int32),
                pltpu.SMEM((1,), jnp.int32),
                pltpu.SemaphoreType.DMA((NR,)),
                pltpu.SemaphoreType.DMA((8,)),
                pltpu.SemaphoreType.DMA((S // DH2,)),
            ] + [pltpu.VMEM((1, S, QB), f32) for _ in range(NSB)]
              + [pltpu.VMEM((1, OFF, QB), f32) for _ in range(NSB)]
              + [pltpu.VMEM((16, QB), f32), pltpu.VMEM((64, QB), u32), pltpu.VMEM((F,), bf16), pltpu.VMEM((D,), bf16)],
            compiler_params=pltpu.CompilerParams(dimension_semantics=("arbitrary",), vmem_limit_bytes=127 * 1024 * 1024),
        )(x, A_wqkv, A_wo, B_w1, B_b1, B_w2, B_b2)
        return out.reshape(1, S, D)
    return fn


_FN = make_kernel()


@jax.jit
def pallas_sequential_preLN__softmax_full_mha__dense_activation_gelu__prompt_kernel(
    A_x: jax.Array,
    A_wqkv: jax.Array,
    A_wo: jax.Array,
    B_x: jax.Array,
    B_w1: jax.Array,
    B_b1: jax.Array,
    B_w2: jax.Array,
    B_b2: jax.Array,
):
    return _FN(A_x, A_wqkv, A_wo, B_x, B_w1, B_b1, B_w2, B_b2)
```

```python
import functools
import math

import jax
import jax.numpy as jnp
from jax import lax
from jax.experimental import pallas as pl
from jax.experimental.pallas import tpu as pltpu

S, D, H, DH, F = 2048, 640, 32, 20, 1536
EPS = 1e-5
QSCALE = (DH ** -0.5) * math.log2(math.e)
NT = (((1,), (1,)), ((), ()))
f32, bf16, u32 = jnp.float32, jnp.bfloat16, jnp.uint32

TSAFE = 60.0
VSC = TSAFE * 2.0 ** -50
LSC = TSAFE * 2.0 ** -60


def _ln(x):
    m = jnp.mean(x, axis=-1, keepdims=True)
    xc = x - m
    v = jnp.mean(xc * xc, axis=-1, keepdims=True)
    return xc * lax.rsqrt(v + EPS)


def make_kernel(FC=256, NCH=4, THIN=2, DP=6):
    TQ, QB, RC, QC, TK = 512, 128, 256, 512, 512
    NC, NQ, NR, NB, NQV = S // TK, S // TQ, S // RC, TQ // QB, S // QC
    NSB = 4
    OFF = 256
    TROWS = (S - OFF) // 16
    NSEG = TROWS // 16
    PPC = OFF // 8 // NC
    KPH, PERQ = 4, 3
    assert KPH + PERQ * NQV == OFF // 16

    def kernel(x_hbm, wqkv_hbm, wo_hbm, w1_hbm, b1_hbm, w2_hbm, b2_hbm, o_hbm,
               x_ref, wqkv_ref, wo_ref, w1_ref, w2_ref, xn_ref,
               kg_ref, qw_ref, vtp_ref, wqvt_ref, m_ref, acc_ref, ot_ref, kb_ref,
               z_ref, ok_ref, xsem, wsem, osem, *rest):
        s_refs = list(zip(rest[:NSB], rest[NSB:2 * NSB]))
        fl_ref, wq_ref, b1_ref, b2_ref = rest[2 * NSB:]
        step = pl.program_id(0)
        z_ref[0] = jnp.minimum(step, 0)
        ob_ref = xn_ref

        def xcopy(r):
            return pltpu.make_async_copy(x_hbm.at[pl.ds(r * RC, RC), :], x_ref.at[pl.ds(r * RC, RC), :], xsem.at[r])

        def wcopy(i):
            if i < 3:
                return pltpu.make_async_copy(wqkv_hbm.at[:, pl.ds(i * D, D)], wqkv_ref.at[i], wsem.at[i])
            src, dst = [(wo_hbm, wo_ref), (w1_hbm, w1_ref), (w2_hbm, w2_ref),
                        (b1_hbm, b1_ref), (b2_hbm, b2_ref)][i - 3]
            return pltpu.make_async_copy(src, dst, wsem.at[i])

        def ocopy(i):
            r0 = i * QB if isinstance(i, int) else pl.multiple_of(i * QB, QB)
            return pltpu.make_async_copy(ob_ref.at[pl.ds(r0, QB), :], o_hbm.at[pl.ds(r0, QB), :], osem.at[i])

        def qprep(h, gq):
            start = h * DH
            g0 = start // 128
            lo = start - g0 * 128
            gi = g0 + 5 if lo + DH > 128 else g0
            a = (lo // 16) * 16
            w = pltpu.bitcast(qw_ref[gq, h], bf16)
            if a + 32 <= 128:
                parts = []
                if a > 0:
                    parts.append(jnp.zeros((a, QB), bf16))
                parts.append(w)
                if a + 32 < 128:
                    parts.append(jnp.zeros((128 - a - 32, QB), bf16))
            else:
                parts = [w[16:32], jnp.zeros((96, QB), bf16), w[0:16]]
            wf = w.astype(f32)
            off = start - (start // 16) * 16
            qrows = [jnp.broadcast_to(wf[off + d:off + d + 1], (8, QB)) for d in range(DH)]
            return gi, jnp.concatenate(parts, axis=0), qrows

        def smpv(h, bufs, m, c, acc, zz):
            s_ref, so_ref = bufs
            sl = slice(c * TK, (c + 1) * TK)
            if c == 0:
                tail = s_ref[zz, TK - 8:TK, :]
                tail = jnp.maximum(tail, jnp.minimum(m, tail))
                sv = jnp.concatenate([so_ref[zz], s_ref[zz, OFF:TK - 8, :], tail], axis=0)
            else:
                sv = s_ref[zz, sl, :]
            p = jnp.exp2(sv).astype(bf16)
            o = jnp.dot(vtp_ref[h, :, sl], p, preferred_element_type=f32)
            return o if acc is None else acc + o

        def finalize(pair, odd, a, lq, keep=None):
            l = a[0:1] if odd else a[23:24]
            r = 1.0 / l
            rows = slice(20, 40) if odd else slice(0, 20)
            a = (a * r)[4:24] if odd else (a * r)[0:20]
            if keep is not None:
                a = jnp.where(keep, a, ot_ref[lq, pair, rows, :])
            ot_ref[lq, pair, rows, :] = a
            return jnp.maximum(l, r)

        def stage(hq, gq, dst, cur, prev):
            sq_ref, so_ref = dst
            gi, qtm, qrows = qprep(hq, gq)
            zz = z_ref[0]
            thin = 1 if hq == H - 1 else THIN
            m8, acc, lr = None, None, None

            def vpu_piece(g):
                parts = []
                for ch in range(NCH):
                    sv = None
                    for d in range(ch, DH, NCH):
                        tt = kb_ref[g, (hq * DH + d) * 8:(hq * DH + d + 1) * 8, :] * qrows[d]
                        sv = tt if sv is None else sv + tt
                    parts.append(sv)
                while len(parts) > 1:
                    parts = [parts[i] + parts[i + 1] if i + 1 < len(parts) else parts[i]
                             for i in range(0, len(parts), 2)]
                so_ref[0, g * 8:(g + 1) * 8, :] = parts[0]
                return parts[0]

            for c in range(NC):
                ss = []
                for u in range(4):
                    lo_ = OFF + (c * 4 + u) * TROWS
                    k = pltpu.bitcast(kg_ref[gi, lo_ // 2:(lo_ + TROWS) // 2, :], bf16)
                    s = jnp.dot(k, qtm, preferred_element_type=f32)
                    sq_ref[0, lo_:lo_ + TROWS, :] = s
                    ss.append(s.reshape(TROWS // 8, 8, QB))
                g = c * PPC
                for qd in range(NSEG):
                    cm = jnp.max(jnp.concatenate([ss[u][2 * qd:2 * qd + 2] for u in range(0, 4, thin)], axis=0), axis=0)
                    m8 = cm if m8 is None else jnp.maximum(m8, cm)
                    for _ in range(1 + (PPC - NSEG if qd == DP else 0)):
                        m8 = jnp.maximum(m8, vpu_piece(g))
                        g += 1
                if c == 0:
                    if prev is not None:
                        hpp, spp, app, lq = prev
                        app = smpv(hpp, spp, None, NC - 1, app, zz)
                        lr = finalize(hpp // 2, hpp % 2 == 1, app, lq)
                elif cur is not None:
                    acc = smpv(cur[0], cur[1], cur[2], c - 1, acc, zz)
            return jnp.max(m8, axis=0, keepdims=True), acc, lr

        @pl.when(step == 0)
        def _prologue():
            xcopy(0).start()
            wcopy(1).start()
            xcopy(1).start()
            for r in range(2, 5):
                xcopy(r).start(priority=1)

            def ln_chunk(r):
                xn_ref[pl.ds(r * RC, RC), :] = _ln(x_ref[pl.ds(r * RC, RC), :].astype(f32)).astype(bf16)

            lane = lax.broadcasted_iota(jnp.int32, (RC // 2, 128), 1)

            def k_chunk(r):
                k = jnp.dot(xn_ref[pl.ds(r * RC, RC), :], wqkv_ref[1], preferred_element_type=f32).astype(bf16)
                k = pltpu.bitcast(k, u32)
                rows = pl.ds(r * RC // 2, RC // 2)
                for g in range(5):
                    kg_ref[g, rows, :] = k[:, 128 * g:128 * (g + 1)]
                for j in range(4):
                    kg_ref[5 + j, rows, :] = jnp.where(lane >= 64, k[:, 128 * j:128 * (j + 1)],
                                                       k[:, 128 * (j + 1):128 * (j + 2)])

            def bcast(i0, n, lanes):
                hb = i0 * 8 if isinstance(i0, int) else pl.multiple_of(i0 * 8, 8)
                kk = jnp.concatenate([kg_ref[g, pl.ds(hb, n * 8), :] for g in range(5)], axis=0)
                for cc in lanes:
                    bb = jnp.broadcast_to(kk[:, cc:cc + 1], (5 * n * 8, 128))
                    bbf = pltpu.bitcast(bb, bf16).astype(f32)
                    for g in range(5):
                        col = g * 128 + cc
                        for gg in range(2 * n):
                            r_ = (g * 2 * n + gg) * 8
                            kb_ref[2 * i0 + gg, col * 8:(col + 1) * 8, :] = bbf[r_:r_ + 8]

            def kb_part(j):
                bcast(0, KPH, range((j * 128) // 7, ((j + 1) * 128) // 7))

            row24 = lax.broadcasted_iota(jnp.int32, (24, QC), 0)
            row32 = lax.broadcasted_iota(jnp.int32, (32, QC), 0)

            def qvbody(r, carry):
                r0 = pl.multiple_of(r * QC, QC)
                qvt = lax.dot_general(wqvt_ref[...].reshape(2 * D, D), xn_ref[pl.ds(r0, QC), :], NT,
                                      preferred_element_type=f32)
                qt = qvt[0:D] * QSCALE
                bcast(KPH + r * PERQ, PERQ, range(128))
                for h in range(H):
                    w0 = (h * DH // 16) * 16
                    off = h * DH - w0
                    w = jnp.where((row32 >= off) & (row32 < off + DH), qt[w0:w0 + 32], 0.0).astype(bf16)
                    w = pltpu.bitcast(w, u32)
                    for j in range(QC // QB):
                        qw_ref[r * (QC // QB) + j, h] = w[:, j * QB:(j + 1) * QB]
                vt = qvt[D:2 * D]
                va = jnp.max(jnp.abs(vt).reshape(D // 8, 8, QC), axis=0)
                va = functools.reduce(jnp.maximum, [va[:, i * 128:(i + 1) * 128] for i in range(QC // 128)])
                fl_ref[8:16, :] = jnp.maximum(fl_ref[8:16, :], va * VSC)
                for h in range(H):
                    w0 = 40 * (h // 2) + 16 * (h % 2)
                    onerow = 0 if h % 2 else 23
                    vtp_ref[h, :, pl.ds(r0, QC)] = jnp.where(row24 == onerow, 1.0, vt[w0:w0 + 24])
                return carry

            s_refs[NSB - 1][0][0, (NC - 1) * TK:, :] = jnp.zeros((TK, QB), f32)
            acc_ref[...] = jnp.ones((24, QB), f32)
            fl_ref[8:16, :] = jnp.zeros((8, QB), f32)

            xcopy(0).wait()
            for r in range(5, 8):
                xcopy(r).start(priority=1)
            ln_chunk(0)
            xcopy(1).wait()
            wcopy(1).wait()
            wcopy(0).start(priority=1)
            wcopy(2).start(priority=1)
            k_chunk(0)
            ln_chunk(1)
            for r in range(2, 5):
                xcopy(r).wait()
            for i in range(3, 8):
                wcopy(i).start(priority=1)
            for r in range(1, 4):
                k_chunk(r)
                kb_part(r - 1)
                ln_chunk(r + 1)
            for r in range(5, 8):
                xcopy(r).wait()
            wcopy(0).wait()
            wcopy(2).wait()
            for r in range(4, 8):
                k_chunk(r)
                kb_part(r - 1)
                if r + 1 < NR:
                    ln_chunk(r + 1)
            wqvt_ref[0] = wqkv_ref[0].T
            wqvt_ref[1] = wqkv_ref[2].T
            lax.fori_loop(0, NQV, qvbody, 0)
            m_ref[0:1, :] = stage(0, 0, s_refs[0], None, None)[0]
            for i in range(3, 8):
                wcopy(i).wait()

        q0 = pl.multiple_of(step * TQ, TQ)
        fl_ref[0:8, :] = fl_ref[8:16, :]

        def bbody(b, carry):
            bp = jnp.where(b == 0, NB - 1, b - 1)
            gq = step * NB + b
            gqn = jnp.minimum(gq + 1, S // QB - 1)
            mp = m_ref[0:1, :]
            app = acc_ref[...]
            lmax, m31 = None, None
            for hp in range(H):
                hq, qq = (hp + 1, gq) if hp + 1 < H else (0, gqn)
                hpp = (hp - 1) % H
                if hp == H - 1:
                    m31 = mp
                mp, app, lr = stage(hq, qq, s_refs[(hp + 1) % NSB],
                                    (hp, s_refs[hp % NSB], mp),
                                    (hpp, s_refs[hpp % NSB], app, b if hp > 0 else bp))
                lmax = lr if lmax is None else jnp.maximum(lmax, lr)
            m_ref[0:1, :] = mp
            acc_ref[...] = app
            fl = jnp.maximum(fl_ref[0:8, :], jnp.maximum(lmax * LSC, jnp.abs(m31)))
            fl_ref[0:8, :] = fl
            ok_ref[0] = jnp.where(jnp.max(fl) <= TSAFE, 1, 0).astype(jnp.int32)
            return carry
        lax.fori_loop(0, NB, bbody, 0)

        ok = ok_ref[0] == 1

        @pl.when(jnp.logical_not(ok))
        def _exact_path():
            sw_ref = s_refs[1][0]

            def one(h, pair, odd, b):
                start = h * DH
                g0 = start // 128
                lo = start - g0 * 128
                gi = jnp.where(lo + DH > 128, g0 + 5, g0)
                a0 = pl.multiple_of((lo // 16) * 8, 8)
                a1 = pl.multiple_of((a0 + 8) % 64, 8)
                w = qw_ref[step * NB + b, h]
                wq_ref[...] = jnp.zeros((64, QB), u32)
                wq_ref[pl.ds(a0, 8), :] = w[0:8]
                wq_ref[pl.ds(a1, 8), :] = w[8:16]
                qtm = pltpu.bitcast(wq_ref[...], bf16)

                def p1(c, m8):
                    k = pltpu.bitcast(kg_ref[gi, pl.ds(pl.multiple_of(c * (TK // 2), TK // 2), TK // 2), :], bf16)
                    s = jnp.dot(k, qtm, preferred_element_type=f32)
                    sw_ref[0, pl.ds(pl.multiple_of(c * TK, TK), TK), :] = s
                    return jnp.maximum(m8, jnp.max(s.reshape(TK // 8, 8, QB), axis=0))
                m8 = lax.fori_loop(0, NC, p1, jnp.full((8, QB), -jnp.inf, f32))
                m = jnp.max(m8, axis=0, keepdims=True)

                def p2(c, acc):
                    r0 = pl.multiple_of(c * TK, TK)
                    p = jnp.exp2(sw_ref[0, pl.ds(r0, TK), :] - m).astype(bf16)
                    return acc + jnp.dot(vtp_ref[h, :, pl.ds(r0, TK)], p, preferred_element_type=f32)
                acc = lax.fori_loop(0, NC, p2, jnp.zeros((24, QB), f32))
                finalize(pair, odd, acc, b)

            def sbody(i, carry):
                b = i // (H // 2)
                pair = i - b * (H // 2)
                one(2 * pair, pair, False, b)
                one(2 * pair + 1, pair, True, b)
                return carry
            lax.fori_loop(0, NB * (H // 2), sbody, 0)

        app = smpv(H - 1, s_refs[(H - 1) % NSB], None, NC - 1, acc_ref[...], z_ref[0])
        finalize((H - 1) // 2, True, app, NB - 1, ok)

        NF = F // FC
        hres, hn = [None] * NB, [None] * NB
        b2 = b2_ref[...].astype(f32)[None, :]
        for a in range(NB):
            o = ot_ref[a].reshape(D, QB).T.astype(bf16)
            hres[a] = (x_ref[pl.ds(q0 + a * QB, QB), :].astype(f32)
                       + jnp.dot(o, wo_ref[...], preferred_element_type=f32))

        def up(a, c):
            if c == 0:
                hn[a] = _ln(hres[a]).astype(bf16)
            u = (jnp.dot(hn[a], w1_ref[:, c * FC:(c + 1) * FC], preferred_element_type=f32)
                 + b1_ref[c * FC:(c + 1) * FC].astype(f32)[None, :])
            return jax.nn.gelu(u, approximate=True).astype(bf16)

        seq = [(a, c) for a in range(NB) for c in range(NF)]
        g = up(*seq[0])
        acc = None
        for i, (a, c) in enumerate(seq):
            gn = up(*seq[i + 1]) if i + 1 < len(seq) else None
            if c == 0:
                acc = hres[a] + b2
            acc = acc + jnp.dot(g, w2_ref[c * FC:(c + 1) * FC, :], preferred_element_type=f32)
            if c == NF - 1:
                ob_ref[pl.ds(q0 + a * QB, QB), :] = acc.astype(bf16)
                ocopy(step * NB + a).start()
            g = gn

        @pl.when(step == NQ - 1)
        def _():
            for i in range(S // QB):
                ocopy(i).wait()

    def fn(A_x, A_wqkv, A_wo, B_x, B_w1, B_b1, B_w2, B_b2):
        x = A_x.reshape(S, D)
        anyspec = pl.BlockSpec(memory_space=pl.ANY)
        out = pl.pallas_call(
            kernel,
            grid=(NQ,),
            in_specs=[anyspec] * 7,
            out_specs=anyspec,
            out_shape=jax.ShapeDtypeStruct((S, D), bf16),
            scratch_shapes=[
                pltpu.VMEM((S, D), bf16),
                pltpu.VMEM((3, D, D), bf16),
                pltpu.VMEM((D, D), bf16),
                pltpu.VMEM((D, F), bf16),
                pltpu.VMEM((F, D), bf16),
                pltpu.VMEM((S, D), bf16),
                pltpu.VMEM((9, S // 2, 128), u32),
                pltpu.VMEM((S // QB, H, 16, QB), u32),
                pltpu.VMEM((H, 24, S), f32),
                pltpu.VMEM((2, D, D), bf16),
                pltpu.VMEM((8, QB), f32),
                pltpu.VMEM((24, QB), f32),
                pltpu.VMEM((NB, H // 2, 40, QB), f32),
                pltpu.VMEM((OFF // 8, D * 8, 128), f32),
                pltpu.SMEM((1,), jnp.int32),
                pltpu.SMEM((1,), jnp.int32),
                pltpu.SemaphoreType.DMA((NR,)),
                pltpu.SemaphoreType.DMA((8,)),
                pltpu.SemaphoreType.DMA((S // QB,)),
            ] + [pltpu.VMEM((1, S, QB), f32) for _ in range(NSB)]
              + [pltpu.VMEM((1, OFF, QB), f32) for _ in range(NSB)]
              + [pltpu.VMEM((16, QB), f32), pltpu.VMEM((64, QB), u32),
                 pltpu.VMEM((F,), bf16), pltpu.VMEM((D,), bf16)],
            compiler_params=pltpu.CompilerParams(dimension_semantics=("arbitrary",),
                                                 vmem_limit_bytes=127 * 1024 * 1024),
        )(x, A_wqkv, A_wo, B_w1, B_b1, B_w2, B_b2)
        return out.reshape(1, S, D)
    return fn


_FN = make_kernel()


@jax.jit
def pallas_sequential_preLN__softmax_full_mha__dense_activation_gelu__prompt_kernel(
    A_x: jax.Array,
    A_wqkv: jax.Array,
    A_wo: jax.Array,
    B_x: jax.Array,
    B_w1: jax.Array,
    B_b1: jax.Array,
    B_w2: jax.Array,
    B_b2: jax.Array,
):
    return _FN(A_x, A_wqkv, A_wo, B_x, B_w1, B_b1, B_w2, B_b2)
```

```python
import functools
import math

import jax
import jax.numpy as jnp
from jax import lax
from jax.experimental import pallas as pl
from jax.experimental.pallas import tpu as pltpu

S, D, H, DH, F = 2048, 640, 32, 20, 1536
EPS = 1e-5
QSCALE = (DH ** -0.5) * math.log2(math.e)
NT = (((1,), (1,)), ((), ()))
f32, bf16, u32 = jnp.float32, jnp.bfloat16, jnp.uint32

TSAFE = 60.0
VSC = TSAFE * 2.0 ** -50
LSC = TSAFE * 2.0 ** -60


def _ln(x):
    m = jnp.mean(x, axis=-1, keepdims=True)
    xc = x - m
    v = jnp.mean(xc * xc, axis=-1, keepdims=True)
    return xc * lax.rsqrt(v + EPS)


def make_kernel(FC=256, NCH=4, THIN=2, DP=6, KM=128):
    TQ, QB, RC, QC, TK = 512, 128, 256, 512, 512
    NC, NQ, NR, NB, NQV = S // TK, S // TQ, S // RC, TQ // QB, S // QC
    NSB = 4
    OFF = 256
    TROWS = (S - OFF) // 16
    NSEG = TROWS // 16
    PPC = OFF // 8 // NC
    KPH, PERQ = 4, 3
    assert KPH + PERQ * NQV == OFF // 16

    def kernel(x_hbm, wqkv_hbm, wo_hbm, w1_hbm, b1_hbm, w2_hbm, b2_hbm, o_hbm,
               x_ref, wqkv_ref, wo_ref, w1_ref, w2_ref, xn_ref,
               kg_ref, qw_ref, vtp_ref, wqvt_ref, m_ref, acc_ref, ot_ref, kb_ref,
               z_ref, ok_ref, xsem, wsem, osem, *rest):
        s_refs = list(zip(rest[:NSB], rest[NSB:2 * NSB]))
        fl_ref, wq_ref, b1_ref, b2_ref = rest[2 * NSB:]
        step = pl.program_id(0)
        z_ref[0] = jnp.minimum(step, 0)
        ob_ref = xn_ref

        def xcopy(r):
            return pltpu.make_async_copy(x_hbm.at[pl.ds(r * RC, RC), :], x_ref.at[pl.ds(r * RC, RC), :], xsem.at[r])

        def wcopy(i):
            if i < 3:
                return pltpu.make_async_copy(wqkv_hbm.at[:, pl.ds(i * D, D)], wqkv_ref.at[i], wsem.at[i])
            src, dst = [(wo_hbm, wo_ref), (w1_hbm, w1_ref), (w2_hbm, w2_ref),
                        (b1_hbm, b1_ref), (b2_hbm, b2_ref)][i - 3]
            return pltpu.make_async_copy(src, dst, wsem.at[i])

        def ocopy(i):
            r0 = i * QB if isinstance(i, int) else pl.multiple_of(i * QB, QB)
            return pltpu.make_async_copy(ob_ref.at[pl.ds(r0, QB), :], o_hbm.at[pl.ds(r0, QB), :], osem.at[i])

        def qprep(h, gq):
            start = h * DH
            g0 = start // 128
            lo = start - g0 * 128
            gi = g0 + 5 if lo + DH > 128 else g0
            a = (lo // 16) * 16
            w = pltpu.bitcast(qw_ref[gq, h], bf16)
            if a + 32 <= 128:
                parts = []
                if a > 0:
                    parts.append(jnp.zeros((a, QB), bf16))
                parts.append(w)
                if a + 32 < 128:
                    parts.append(jnp.zeros((128 - a - 32, QB), bf16))
            else:
                parts = [w[16:32], jnp.zeros((96, QB), bf16), w[0:16]]
            wf = w.astype(f32)
            off = start - (start // 16) * 16
            qrows = [jnp.broadcast_to(wf[off + d:off + d + 1], (8, QB)) for d in range(DH)]
            return gi, jnp.concatenate(parts, axis=0), qrows

        def smpv(h, bufs, m, c, acc, zz):
            s_ref, so_ref = bufs
            sl = slice(c * TK, (c + 1) * TK)
            if c == 0:
                tail = s_ref[zz, TK - 8:TK, :]
                tail = jnp.maximum(tail, jnp.minimum(m, tail))
                sv = jnp.concatenate([so_ref[zz], s_ref[zz, OFF:TK - 8, :], tail], axis=0)
            else:
                sv = s_ref[zz, sl, :]
            p = jnp.exp2(sv).astype(bf16)
            o = jnp.dot(vtp_ref[h, :, sl], p, preferred_element_type=f32)
            return o if acc is None else acc + o

        def finalize(pair, odd, a, lq, keep=None):
            l = a[0:1] if odd else a[23:24]
            r = 1.0 / l
            rows = slice(20, 40) if odd else slice(0, 20)
            a = (a * r)[4:24] if odd else (a * r)[0:20]
            if keep is not None:
                a = jnp.where(keep, a, ot_ref[lq, pair, rows, :])
            ot_ref[lq, pair, rows, :] = a
            return jnp.maximum(l, r)

        def stage(hq, gq, dst, cur, prev):
            sq_ref, so_ref = dst
            gi, qtm, qrows = qprep(hq, gq)
            zz = z_ref[0]
            thin = 1 if hq == H - 1 else THIN
            m8, acc, lr = None, None, None

            def vpu_piece(g):
                parts = []
                for ch in range(NCH):
                    sv = None
                    for d in range(ch, DH, NCH):
                        tt = kb_ref[g, (hq * DH + d) * 8:(hq * DH + d + 1) * 8, :] * qrows[d]
                        sv = tt if sv is None else sv + tt
                    parts.append(sv)
                while len(parts) > 1:
                    parts = [parts[i] + parts[i + 1] if i + 1 < len(parts) else parts[i]
                             for i in range(0, len(parts), 2)]
                so_ref[0, g * 8:(g + 1) * 8, :] = parts[0]
                return parts[0]

            for c in range(NC):
                ss = []
                for u in range(4):
                    lo_ = OFF + (c * 4 + u) * TROWS
                    k = pltpu.bitcast(kg_ref[gi, lo_ // 2:(lo_ + TROWS) // 2, :], bf16)
                    s = jnp.dot(k, qtm, preferred_element_type=f32)
                    sq_ref[0, lo_:lo_ + TROWS, :] = s
                    ss.append(s.reshape(TROWS // 8, 8, QB))
                g = c * PPC
                for qd in range(NSEG):
                    cm = jnp.max(jnp.concatenate([ss[u][2 * qd:2 * qd + 2] for u in range(0, 4, thin)], axis=0), axis=0)
                    m8 = cm if m8 is None else jnp.maximum(m8, cm)
                    for _ in range(1 + (PPC - NSEG if qd == DP else 0)):
                        m8 = jnp.maximum(m8, vpu_piece(g))
                        g += 1
                if c == 0:
                    if prev is not None:
                        hpp, spp, app, lq = prev
                        app = smpv(hpp, spp, None, NC - 1, app, zz)
                        lr = finalize(hpp // 2, hpp % 2 == 1, app, lq)
                elif cur is not None:
                    acc = smpv(cur[0], cur[1], cur[2], c - 1, acc, zz)
            return jnp.max(m8, axis=0, keepdims=True), acc, lr

        @pl.when(step == 0)
        def _prologue():
            xcopy(0).start()
            wcopy(1).start()
            xcopy(1).start()
            for r in range(2, 5):
                xcopy(r).start(priority=1)

            def ln_chunk(r):
                xn_ref[pl.ds(r * RC, RC), :] = _ln(x_ref[pl.ds(r * RC, RC), :].astype(f32)).astype(bf16)

            lane = lax.broadcasted_iota(jnp.int32, (KM // 2, 128), 1)

            def k_chunk(r):
                for r0 in range(r * RC, (r + 1) * RC, KM):
                    k = jnp.dot(xn_ref[pl.ds(r0, KM), :], wqkv_ref[1], preferred_element_type=f32).astype(bf16)
                    k = pltpu.bitcast(k, u32)
                    rows = pl.ds(r0 // 2, KM // 2)
                    for g in range(5):
                        kg_ref[g, rows, :] = k[:, 128 * g:128 * (g + 1)]
                    for j in range(4):
                        kg_ref[5 + j, rows, :] = jnp.where(lane >= 64, k[:, 128 * j:128 * (j + 1)],
                                                           k[:, 128 * (j + 1):128 * (j + 2)])

            def bcast(i0, n, lanes):
                hb = i0 * 8 if isinstance(i0, int) else pl.multiple_of(i0 * 8, 8)
                kk = jnp.concatenate([kg_ref[g, pl.ds(hb, n * 8), :] for g in range(5)], axis=0)
                for cc in lanes:
                    bb = jnp.broadcast_to(kk[:, cc:cc + 1], (5 * n * 8, 128))
                    bbf = pltpu.bitcast(bb, bf16).astype(f32)
                    for g in range(5):
                        col = g * 128 + cc
                        for gg in range(2 * n):
                            r_ = (g * 2 * n + gg) * 8
                            kb_ref[2 * i0 + gg, col * 8:(col + 1) * 8, :] = bbf[r_:r_ + 8]

            WT = [2, 2, 1, 2, 2, 2, 1]
            cum = [sum(WT[:i_]) for i_ in range(8)]

            def kb_part(j):
                bcast(0, KPH, range((cum[j] * 128) // cum[7], (cum[j + 1] * 128) // cum[7]))

            row24 = lax.broadcasted_iota(jnp.int32, (24, QC), 0)
            row32 = lax.broadcasted_iota(jnp.int32, (32, QC), 0)

            def qvbody(r, carry):
                r0 = pl.multiple_of(r * QC, QC)
                qvt = lax.dot_general(wqvt_ref[...].reshape(2 * D, D), xn_ref[pl.ds(r0, QC), :], NT,
                                      preferred_element_type=f32)
                qt = qvt[0:D] * QSCALE
                bcast(KPH + r * PERQ, PERQ, range(128))
                for h in range(H):
                    w0 = (h * DH // 16) * 16
                    off = h * DH - w0
                    w = jnp.where((row32 >= off) & (row32 < off + DH), qt[w0:w0 + 32], 0.0).astype(bf16)
                    w = pltpu.bitcast(w, u32)
                    for j in range(QC // QB):
                        qw_ref[r * (QC // QB) + j, h] = w[:, j * QB:(j + 1) * QB]
                vt = qvt[D:2 * D]
                va = jnp.max(jnp.abs(vt).reshape(D // 8, 8, QC), axis=0)
                va = functools.reduce(jnp.maximum, [va[:, i * 128:(i + 1) * 128] for i in range(QC // 128)])
                fl_ref[8:16, :] = jnp.maximum(fl_ref[8:16, :], va * VSC)
                for h in range(H):
                    w0 = 40 * (h // 2) + 16 * (h % 2)
                    onerow = 0 if h % 2 else 23
                    vtp_ref[h, :, pl.ds(r0, QC)] = jnp.where(row24 == onerow, 1.0, vt[w0:w0 + 24])
                return carry

            s_refs[NSB - 1][0][0, (NC - 1) * TK:, :] = jnp.zeros((TK, QB), f32)
            acc_ref[...] = jnp.ones((24, QB), f32)
            fl_ref[8:16, :] = jnp.zeros((8, QB), f32)

            xcopy(0).wait()
            for r in range(5, 8):
                xcopy(r).start(priority=1)
            ln_chunk(0)
            xcopy(1).wait()
            wcopy(1).wait()
            wcopy(0).start(priority=1)
            wcopy(2).start(priority=1)
            k_chunk(0)
            ln_chunk(1)
            for r in range(2, 5):
                xcopy(r).wait()
            for i in range(3, 8):
                wcopy(i).start(priority=1)
            for r in range(1, 4):
                k_chunk(r)
                kb_part(r - 1)
                ln_chunk(r + 1)
            for r in range(5, 8):
                xcopy(r).wait()
            wcopy(0).wait()
            wcopy(2).wait()
            for r in range(4, 8):
                k_chunk(r)
                kb_part(r - 1)
                if r + 1 < NR:
                    ln_chunk(r + 1)
            wqvt_ref[0] = wqkv_ref[0].T
            wqvt_ref[1] = wqkv_ref[2].T
            lax.fori_loop(0, NQV, qvbody, 0)
            m_ref[0:1, :] = stage(0, 0, s_refs[0], None, None)[0]
            for i in range(3, 8):
                wcopy(i).wait()

        q0 = pl.multiple_of(step * TQ, TQ)
        fl_ref[0:8, :] = fl_ref[8:16, :]

        def bbody(b, carry):
            bp = jnp.where(b == 0, NB - 1, b - 1)
            gq = step * NB + b
            gqn = jnp.minimum(gq + 1, S // QB - 1)
            mp = m_ref[0:1, :]
            app = acc_ref[...]
            lmax, m31 = None, None
            for hp in range(H):
                hq, qq = (hp + 1, gq) if hp + 1 < H else (0, gqn)
                hpp = (hp - 1) % H
                if hp == H - 1:
                    m31 = mp
                mp, app, lr = stage(hq, qq, s_refs[(hp + 1) % NSB],
                                    (hp, s_refs[hp % NSB], mp),
                                    (hpp, s_refs[hpp % NSB], app, b if hp > 0 else bp))
                lmax = lr if lmax is None else jnp.maximum(lmax, lr)
            m_ref[0:1, :] = mp
            acc_ref[...] = app
            fl = jnp.maximum(fl_ref[0:8, :], jnp.maximum(lmax * LSC, jnp.abs(m31)))
            fl_ref[0:8, :] = fl
            ok_ref[0] = jnp.where(jnp.max(fl) <= TSAFE, 1, 0).astype(jnp.int32)
            return carry
        lax.fori_loop(0, NB, bbody, 0)

        ok = ok_ref[0] == 1

        @pl.when(jnp.logical_not(ok))
        def _exact_path():
            sw_ref = s_refs[1][0]

            def one(h, pair, odd, b):
                start = h * DH
                g0 = start // 128
                lo = start - g0 * 128
                gi = jnp.where(lo + DH > 128, g0 + 5, g0)
                a0 = pl.multiple_of((lo // 16) * 8, 8)
                a1 = pl.multiple_of((a0 + 8) % 64, 8)
                w = qw_ref[step * NB + b, h]
                wq_ref[...] = jnp.zeros((64, QB), u32)
                wq_ref[pl.ds(a0, 8), :] = w[0:8]
                wq_ref[pl.ds(a1, 8), :] = w[8:16]
                qtm = pltpu.bitcast(wq_ref[...], bf16)

                def p1(c, m8):
                    k = pltpu.bitcast(kg_ref[gi, pl.ds(pl.multiple_of(c * (TK // 2), TK // 2), TK // 2), :], bf16)
                    s = jnp.dot(k, qtm, preferred_element_type=f32)
                    sw_ref[0, pl.ds(pl.multiple_of(c * TK, TK), TK), :] = s
                    return jnp.maximum(m8, jnp.max(s.reshape(TK // 8, 8, QB), axis=0))
                m8 = lax.fori_loop(0, NC, p1, jnp.full((8, QB), -jnp.inf, f32))
                m = jnp.max(m8, axis=0, keepdims=True)

                def p2(c, acc):
                    r0 = pl.multiple_of(c * TK, TK)
                    p = jnp.exp2(sw_ref[0, pl.ds(r0, TK), :] - m).astype(bf16)
                    return acc + jnp.dot(vtp_ref[h, :, pl.ds(r0, TK)], p, preferred_element_type=f32)
                acc = lax.fori_loop(0, NC, p2, jnp.zeros((24, QB), f32))
                finalize(pair, odd, acc, b)

            def sbody(i, carry):
                b = i // (H // 2)
                pair = i - b * (H // 2)
                one(2 * pair, pair, False, b)
                one(2 * pair + 1, pair, True, b)
                return carry
            lax.fori_loop(0, NB * (H // 2), sbody, 0)

        app = smpv(H - 1, s_refs[(H - 1) % NSB], None, NC - 1, acc_ref[...], z_ref[0])
        finalize((H - 1) // 2, True, app, NB - 1, ok)

        NF = F // FC
        hres, hn = [None] * NB, [None] * NB
        b2 = b2_ref[...].astype(f32)[None, :]
        for a in range(NB):
            o = ot_ref[a].reshape(D, QB).T.astype(bf16)
            hres[a] = (x_ref[pl.ds(q0 + a * QB, QB), :].astype(f32)
                       + jnp.dot(o, wo_ref[...], preferred_element_type=f32))

        def up(a, c):
            if c == 0:
                hn[a] = _ln(hres[a]).astype(bf16)
            u = (jnp.dot(hn[a], w1_ref[:, c * FC:(c + 1) * FC], preferred_element_type=f32)
                 + b1_ref[c * FC:(c + 1) * FC].astype(f32)[None, :])
            return jax.nn.gelu(u, approximate=True).astype(bf16)

        seq = [(a, c) for a in range(NB) for c in range(NF)]
        g = up(*seq[0])
        acc = None
        for i, (a, c) in enumerate(seq):
            gn = up(*seq[i + 1]) if i + 1 < len(seq) else None
            if c == 0:
                acc = hres[a] + b2
            acc = acc + jnp.dot(g, w2_ref[c * FC:(c + 1) * FC, :], preferred_element_type=f32)
            if c == NF - 1:
                ob_ref[pl.ds(q0 + a * QB, QB), :] = acc.astype(bf16)
                ocopy(step * NB + a).start()
            g = gn

        @pl.when(step == NQ - 1)
        def _():
            for i in range(S // QB):
                ocopy(i).wait()

    def fn(A_x, A_wqkv, A_wo, B_x, B_w1, B_b1, B_w2, B_b2):
        x = A_x.reshape(S, D)
        anyspec = pl.BlockSpec(memory_space=pl.ANY)
        out = pl.pallas_call(
            kernel,
            grid=(NQ,),
            in_specs=[anyspec] * 7,
            out_specs=anyspec,
            out_shape=jax.ShapeDtypeStruct((S, D), bf16),
            scratch_shapes=[
                pltpu.VMEM((S, D), bf16),
                pltpu.VMEM((3, D, D), bf16),
                pltpu.VMEM((D, D), bf16),
                pltpu.VMEM((D, F), bf16),
                pltpu.VMEM((F, D), bf16),
                pltpu.VMEM((S, D), bf16),
                pltpu.VMEM((9, S // 2, 128), u32),
                pltpu.VMEM((S // QB, H, 16, QB), u32),
                pltpu.VMEM((H, 24, S), f32),
                pltpu.VMEM((2, D, D), bf16),
                pltpu.VMEM((8, QB), f32),
                pltpu.VMEM((24, QB), f32),
                pltpu.VMEM((NB, H // 2, 40, QB), f32),
                pltpu.VMEM((OFF // 8, D * 8, 128), f32),
                pltpu.SMEM((1,), jnp.int32),
                pltpu.SMEM((1,), jnp.int32),
                pltpu.SemaphoreType.DMA((NR,)),
                pltpu.SemaphoreType.DMA((8,)),
                pltpu.SemaphoreType.DMA((S // QB,)),
            ] + [pltpu.VMEM((1, S, QB), f32) for _ in range(NSB)]
              + [pltpu.VMEM((1, OFF, QB), f32) for _ in range(NSB)]
              + [pltpu.VMEM((16, QB), f32), pltpu.VMEM((64, QB), u32),
                 pltpu.VMEM((F,), bf16), pltpu.VMEM((D,), bf16)],
            compiler_params=pltpu.CompilerParams(dimension_semantics=("arbitrary",),
                                                 vmem_limit_bytes=127 * 1024 * 1024),
        )(x, A_wqkv, A_wo, B_w1, B_b1, B_w2, B_b2)
        return out.reshape(1, S, D)
    return fn


_FN = make_kernel()


@jax.jit
def pallas_sequential_preLN__softmax_full_mha__dense_activation_gelu__prompt_kernel(
    A_x: jax.Array,
    A_wqkv: jax.Array,
    A_wo: jax.Array,
    B_x: jax.Array,
    B_w1: jax.Array,
    B_b1: jax.Array,
    B_w2: jax.Array,
    B_b2: jax.Array,
):
    return _FN(A_x, A_wqkv, A_wo, B_x, B_w1, B_b1, B_w2, B_b2)
```

```python
import functools
import math

import jax
import jax.numpy as jnp
from jax import lax
from jax.experimental import pallas as pl
from jax.experimental.pallas import tpu as pltpu

S, D, H, DH, F = 2048, 640, 32, 20, 1536
EPS = 1e-5
QSCALE = (DH ** -0.5) * math.log2(math.e)
NT = (((1,), (1,)), ((), ()))
f32, bf16, u32 = jnp.float32, jnp.bfloat16, jnp.uint32

TSAFE = 60.0
VSC = TSAFE * 2.0 ** -50
LSC = TSAFE * 2.0 ** -60


def _ln(x):
    m = jnp.mean(x, axis=-1, keepdims=True)
    xc = x - m
    v = jnp.mean(xc * xc, axis=-1, keepdims=True)
    return xc * lax.rsqrt(v + EPS)


def make_kernel(FC=256, THIN=2, DP=6, KM=128):
    TQ, QB, RC, QC, TK = 512, 128, 256, 512, 512
    NC, NQ, NR, NB, NQV = S // TK, S // TQ, S // RC, TQ // QB, S // QC
    NSB = 4
    OFF = 256
    TROWS = (S - OFF) // 16
    NSEG = TROWS // 16
    PPC = OFF // 8 // NC
    KPH, PERQ = 4, 3
    assert KPH + PERQ * NQV == OFF // 16

    def kernel(x_hbm, wqkv_hbm, wo_hbm, w1_hbm, b1_hbm, w2_hbm, b2_hbm, o_hbm,
               x_ref, wqkv_ref, wo_ref, w1_ref, w2_ref, xn_ref,
               kg_ref, qw_ref, vtp_ref, wqvt_ref, m_ref, acc_ref, ot_ref, kb_ref,
               z_ref, ok_ref, xsem, wsem, osem, *rest):
        s_refs = list(zip(rest[:NSB], rest[NSB:2 * NSB]))
        fl_ref, wq_ref, b1_ref, b2_ref = rest[2 * NSB:]
        step = pl.program_id(0)
        z_ref[0] = jnp.minimum(step, 0)
        ob_ref = xn_ref

        def xcopy(r):
            return pltpu.make_async_copy(x_hbm.at[pl.ds(r * RC, RC), :], x_ref.at[pl.ds(r * RC, RC), :], xsem.at[r])

        def wcopy(i):
            if i < 3:
                return pltpu.make_async_copy(wqkv_hbm.at[:, pl.ds(i * D, D)], wqkv_ref.at[i], wsem.at[i])
            src, dst = [(wo_hbm, wo_ref), (w1_hbm, w1_ref), (w2_hbm, w2_ref),
                        (b1_hbm, b1_ref), (b2_hbm, b2_ref)][i - 3]
            return pltpu.make_async_copy(src, dst, wsem.at[i])

        def ocopy(i):
            r0 = i * QB if isinstance(i, int) else pl.multiple_of(i * QB, QB)
            return pltpu.make_async_copy(ob_ref.at[pl.ds(r0, QB), :], o_hbm.at[pl.ds(r0, QB), :], osem.at[i])

        def qprep(h, gq):
            start = h * DH
            g0 = start // 128
            lo = start - g0 * 128
            gi = g0 + 5 if lo + DH > 128 else g0
            a = (lo // 16) * 16
            w = pltpu.bitcast(qw_ref[gq, h], bf16)
            if a + 32 <= 128:
                parts = []
                if a > 0:
                    parts.append(jnp.zeros((a, QB), bf16))
                parts.append(w)
                if a + 32 < 128:
                    parts.append(jnp.zeros((128 - a - 32, QB), bf16))
            else:
                parts = [w[16:32], jnp.zeros((96, QB), bf16), w[0:16]]
            wf = w.astype(f32)
            off = start - (start // 16) * 16
            qrows = jnp.stack([jnp.broadcast_to(wf[off + d:off + d + 1], (8, QB)) for d in range(DH)])
            qrows = qrows.reshape(DH // 4, 2, 2, 8, QB)
            return gi, jnp.concatenate(parts, axis=0), qrows

        def smpv(h, bufs, m, c, acc, zz):
            s_ref, so_ref = bufs
            sl = slice(c * TK, (c + 1) * TK)
            if c == 0:
                tail = s_ref[zz, TK - 8:TK, :]
                tail = jnp.maximum(tail, jnp.minimum(m, tail))
                sv = jnp.concatenate([so_ref[zz], s_ref[zz, OFF:TK - 8, :], tail], axis=0)
            else:
                sv = s_ref[zz, sl, :]
            p = jnp.exp2(sv).astype(bf16)
            o = jnp.dot(vtp_ref[h, :, sl], p, preferred_element_type=f32)
            return o if acc is None else acc + o

        def finalize(pair, odd, a, lq, keep=None):
            l = a[0:1] if odd else a[23:24]
            r = 1.0 / l
            rows = slice(20, 40) if odd else slice(0, 20)
            a = (a * r)[4:24] if odd else (a * r)[0:20]
            if keep is not None:
                a = jnp.where(keep, a, ot_ref[lq, pair, rows, :])
            ot_ref[lq, pair, rows, :] = a
            return jnp.maximum(l, r)

        def stage(hq, gq, dst, cur, prev):
            sq_ref, so_ref = dst
            gi, qtm, qrows = qprep(hq, gq)
            zz = z_ref[0]
            thin = 1 if hq == H - 1 else THIN
            m8, acc, lr = None, None, None

            def vpu_piece(g):
                kb = kb_ref[g, hq * DH * 8:(hq + 1) * DH * 8, :].reshape(DH // 4, 2, 2, 8, QB)
                sv = jnp.sum(jnp.sum(jnp.sum(kb * qrows, axis=0), axis=1), axis=0)
                so_ref[0, g * 8:(g + 1) * 8, :] = sv
                return sv

            for c in range(NC):
                ss = []
                for u in range(4):
                    lo_ = OFF + (c * 4 + u) * TROWS
                    k = pltpu.bitcast(kg_ref[gi, lo_ // 2:(lo_ + TROWS) // 2, :], bf16)
                    s = jnp.dot(k, qtm, preferred_element_type=f32)
                    sq_ref[0, lo_:lo_ + TROWS, :] = s
                    ss.append(s.reshape(TROWS // 8, 8, QB))
                g = c * PPC
                for qd in range(NSEG):
                    cm = jnp.max(jnp.concatenate([ss[u][2 * qd:2 * qd + 2] for u in range(0, 4, thin)], axis=0), axis=0)
                    m8 = cm if m8 is None else jnp.maximum(m8, cm)
                    for _ in range(1 + (PPC - NSEG if qd == DP else 0)):
                        m8 = jnp.maximum(m8, vpu_piece(g))
                        g += 1
                if c == 0:
                    if prev is not None:
                        hpp, spp, app, lq = prev
                        app = smpv(hpp, spp, None, NC - 1, app, zz)
                        lr = finalize(hpp // 2, hpp % 2 == 1, app, lq)
                elif cur is not None:
                    acc = smpv(cur[0], cur[1], cur[2], c - 1, acc, zz)
            return jnp.max(m8, axis=0, keepdims=True), acc, lr

        @pl.when(step == 0)
        def _prologue():
            xcopy(0).start()
            wcopy(1).start()
            xcopy(1).start()
            for r in range(2, 5):
                xcopy(r).start(priority=1)

            def ln_chunk(r):
                xn_ref[pl.ds(r * RC, RC), :] = _ln(x_ref[pl.ds(r * RC, RC), :].astype(f32)).astype(bf16)

            lane = lax.broadcasted_iota(jnp.int32, (KM // 2, 128), 1)

            def k_chunk(r):
                for r0 in range(r * RC, (r + 1) * RC, KM):
                    k = jnp.dot(xn_ref[pl.ds(r0, KM), :], wqkv_ref[1], preferred_element_type=f32).astype(bf16)
                    k = pltpu.bitcast(k, u32)
                    rows = pl.ds(r0 // 2, KM // 2)
                    for g in range(5):
                        kg_ref[g, rows, :] = k[:, 128 * g:128 * (g + 1)]
                    for j in range(4):
                        kg_ref[5 + j, rows, :] = jnp.where(lane >= 64, k[:, 128 * j:128 * (j + 1)],
                                                           k[:, 128 * (j + 1):128 * (j + 2)])

            def bcast(i0, n, lanes):
                hb = i0 * 8 if isinstance(i0, int) else pl.multiple_of(i0 * 8, 8)
                kk = jnp.concatenate([kg_ref[g, pl.ds(hb, n * 8), :] for g in range(5)], axis=0)
                for cc in lanes:
                    bb = jnp.broadcast_to(kk[:, cc:cc + 1], (5 * n * 8, 128))
                    bbf = pltpu.bitcast(bb, bf16).astype(f32).reshape(5, 2 * n, 8, 128)
                    for g in range(5):
                        col = g * 128 + cc
                        kb_ref[pl.ds(2 * i0, 2 * n), col * 8:(col + 1) * 8, :] = bbf[g]

            WT = [2, 2, 1, 2, 2, 2, 1]
            cum = [sum(WT[:i_]) for i_ in range(8)]

            def kb_part(j):
                bcast(0, KPH, range((cum[j] * 128) // cum[7], (cum[j + 1] * 128) // cum[7]))

            row24 = lax.broadcasted_iota(jnp.int32, (24, QC), 0)
            row32 = lax.broadcasted_iota(jnp.int32, (32, QC), 0)

            def qvbody(r, carry):
                r0 = pl.multiple_of(r * QC, QC)
                qvt = lax.dot_general(wqvt_ref[...].reshape(2 * D, D), xn_ref[pl.ds(r0, QC), :], NT,
                                      preferred_element_type=f32)
                qt = qvt[0:D] * QSCALE
                bcast(KPH + r * PERQ, PERQ, range(128))
                for h in range(H):
                    w0 = (h * DH // 16) * 16
                    off = h * DH - w0
                    w = jnp.where((row32 >= off) & (row32 < off + DH), qt[w0:w0 + 32], 0.0).astype(bf16)
                    w = pltpu.bitcast(w, u32)
                    for j in range(QC // QB):
                        qw_ref[r * (QC // QB) + j, h] = w[:, j * QB:(j + 1) * QB]
                vt = qvt[D:2 * D]
                va = jnp.max(jnp.abs(vt).reshape(D // 8, 8, QC), axis=0)
                va = functools.reduce(jnp.maximum, [va[:, i * 128:(i + 1) * 128] for i in range(QC // 128)])
                fl_ref[8:16, :] = jnp.maximum(fl_ref[8:16, :], va * VSC)
                for h in range(H):
                    w0 = 40 * (h // 2) + 16 * (h % 2)
                    onerow = 0 if h % 2 else 23
                    vtp_ref[h, :, pl.ds(r0, QC)] = jnp.where(row24 == onerow, 1.0, vt[w0:w0 + 24])
                return carry

            s_refs[NSB - 1][0][0, (NC - 1) * TK:, :] = jnp.zeros((TK, QB), f32)
            acc_ref[...] = jnp.ones((24, QB), f32)
            fl_ref[8:16, :] = jnp.zeros((8, QB), f32)

            xcopy(0).wait()
            for r in range(5, 8):
                xcopy(r).start(priority=1)
            ln_chunk(0)
            xcopy(1).wait()
            wcopy(1).wait()
            wcopy(0).start(priority=1)
            wcopy(2).start(priority=1)
            k_chunk(0)
            ln_chunk(1)
            for r in range(2, 5):
                xcopy(r).wait()
            for i in range(3, 8):
                wcopy(i).start(priority=1)
            for r in range(1, 4):
                k_chunk(r)
                kb_part(r - 1)
                ln_chunk(r + 1)
            for r in range(5, 8):
                xcopy(r).wait()
            wcopy(0).wait()
            wcopy(2).wait()
            for r in range(4, 8):
                k_chunk(r)
                kb_part(r - 1)
                if r + 1 < NR:
                    ln_chunk(r + 1)
            wqvt_ref[0] = wqkv_ref[0].T
            wqvt_ref[1] = wqkv_ref[2].T
            lax.fori_loop(0, NQV, qvbody, 0)
            m_ref[0:1, :] = stage(0, 0, s_refs[0], None, None)[0]
            for i in range(3, 8):
                wcopy(i).wait()

        q0 = pl.multiple_of(step * TQ, TQ)
        fl_ref[0:8, :] = fl_ref[8:16, :]

        def bbody(b, carry):
            bp = jnp.where(b == 0, NB - 1, b - 1)
            gq = step * NB + b
            gqn = jnp.minimum(gq + 1, S // QB - 1)
            mp = m_ref[0:1, :]
            app = acc_ref[...]
            lmax, m31 = None, None
            for hp in range(H):
                hq, qq = (hp + 1, gq) if hp + 1 < H else (0, gqn)
                hpp = (hp - 1) % H
                if hp == H - 1:
                    m31 = mp
                mp, app, lr = stage(hq, qq, s_refs[(hp + 1) % NSB],
                                    (hp, s_refs[hp % NSB], mp),
                                    (hpp, s_refs[hpp % NSB], app, b if hp > 0 else bp))
                lmax = lr if lmax is None else jnp.maximum(lmax, lr)
            m_ref[0:1, :] = mp
            acc_ref[...] = app
            fl = jnp.maximum(fl_ref[0:8, :], jnp.maximum(lmax * LSC, jnp.abs(m31)))
            fl_ref[0:8, :] = fl
            ok_ref[0] = jnp.where(jnp.max(fl) <= TSAFE, 1, 0).astype(jnp.int32)
            return carry
        lax.fori_loop(0, NB, bbody, 0)

        ok = ok_ref[0] == 1

        @pl.when(jnp.logical_not(ok))
        def _exact_path():
            sw_ref = s_refs[1][0]

            def one(h, pair, odd, b):
                start = h * DH
                g0 = start // 128
                lo = start - g0 * 128
                gi = jnp.where(lo + DH > 128, g0 + 5, g0)
                a0 = pl.multiple_of((lo // 16) * 8, 8)
                a1 = pl.multiple_of((a0 + 8) % 64, 8)
                w = qw_ref[step * NB + b, h]
                wq_ref[...] = jnp.zeros((64, QB), u32)
                wq_ref[pl.ds(a0, 8), :] = w[0:8]
                wq_ref[pl.ds(a1, 8), :] = w[8:16]
                qtm = pltpu.bitcast(wq_ref[...], bf16)

                def p1(c, m8):
                    k = pltpu.bitcast(kg_ref[gi, pl.ds(pl.multiple_of(c * (TK // 2), TK // 2), TK // 2), :], bf16)
                    s = jnp.dot(k, qtm, preferred_element_type=f32)
                    sw_ref[0, pl.ds(pl.multiple_of(c * TK, TK), TK), :] = s
                    return jnp.maximum(m8, jnp.max(s.reshape(TK // 8, 8, QB), axis=0))
                m8 = lax.fori_loop(0, NC, p1, jnp.full((8, QB), -jnp.inf, f32))
                m = jnp.max(m8, axis=0, keepdims=True)

                def p2(c, acc):
                    r0 = pl.multiple_of(c * TK, TK)
                    p = jnp.exp2(sw_ref[0, pl.ds(r0, TK), :] - m).astype(bf16)
                    return acc + jnp.dot(vtp_ref[h, :, pl.ds(r0, TK)], p, preferred_element_type=f32)
                acc = lax.fori_loop(0, NC, p2, jnp.zeros((24, QB), f32))
                finalize(pair, odd, acc, b)

            def sbody(i, carry):
                b = i // (H // 2)
                pair = i - b * (H // 2)
                one(2 * pair, pair, False, b)
                one(2 * pair + 1, pair, True, b)
                return carry
            lax.fori_loop(0, NB * (H // 2), sbody, 0)

        app = smpv(H - 1, s_refs[(H - 1) % NSB], None, NC - 1, acc_ref[...], z_ref[0])
        finalize((H - 1) // 2, True, app, NB - 1, ok)

        NF = F // FC
        hres, hn = [None] * NB, [None] * NB
        b2 = b2_ref[...].astype(f32)[None, :]
        for a in range(NB):
            o = ot_ref[a].reshape(D, QB).T.astype(bf16)
            hres[a] = (x_ref[pl.ds(q0 + a * QB, QB), :].astype(f32)
                       + jnp.dot(o, wo_ref[...], preferred_element_type=f32))

        def up(a, c):
            if c == 0:
                hn[a] = _ln(hres[a]).astype(bf16)
            u = (jnp.dot(hn[a], w1_ref[:, c * FC:(c + 1) * FC], preferred_element_type=f32)
                 + b1_ref[c * FC:(c + 1) * FC].astype(f32)[None, :])
            return jax.nn.gelu(u, approximate=True).astype(bf16)

        seq = [(a, c) for a in range(NB) for c in range(NF)]
        g = up(*seq[0])
        acc = None
        for i, (a, c) in enumerate(seq):
            gn = up(*seq[i + 1]) if i + 1 < len(seq) else None
            if c == 0:
                acc = hres[a] + b2
            acc = acc + jnp.dot(g, w2_ref[c * FC:(c + 1) * FC, :], preferred_element_type=f32)
            if c == NF - 1:
                ob_ref[pl.ds(q0 + a * QB, QB), :] = acc.astype(bf16)
                ocopy(step * NB + a).start()
            g = gn

        @pl.when(step == NQ - 1)
        def _():
            for i in range(S // QB):
                ocopy(i).wait()

    def fn(A_x, A_wqkv, A_wo, B_x, B_w1, B_b1, B_w2, B_b2):
        x = A_x.reshape(S, D)
        anyspec = pl.BlockSpec(memory_space=pl.ANY)
        out = pl.pallas_call(
            kernel,
            grid=(NQ,),
            in_specs=[anyspec] * 7,
            out_specs=anyspec,
            out_shape=jax.ShapeDtypeStruct((S, D), bf16),
            scratch_shapes=[
                pltpu.VMEM((S, D), bf16),
                pltpu.VMEM((3, D, D), bf16),
                pltpu.VMEM((D, D), bf16),
                pltpu.VMEM((D, F), bf16),
                pltpu.VMEM((F, D), bf16),
                pltpu.VMEM((S, D), bf16),
                pltpu.VMEM((9, S // 2, 128), u32),
                pltpu.VMEM((S // QB, H, 16, QB), u32),
                pltpu.VMEM((H, 24, S), f32),
                pltpu.VMEM((2, D, D), bf16),
                pltpu.VMEM((8, QB), f32),
                pltpu.VMEM((24, QB), f32),
                pltpu.VMEM((NB, H // 2, 40, QB), f32),
                pltpu.VMEM((OFF // 8, D * 8, 128), f32),
                pltpu.SMEM((1,), jnp.int32),
                pltpu.SMEM((1,), jnp.int32),
                pltpu.SemaphoreType.DMA((NR,)),
                pltpu.SemaphoreType.DMA((8,)),
                pltpu.SemaphoreType.DMA((S // QB,)),
            ] + [pltpu.VMEM((1, S, QB), f32) for _ in range(NSB)]
              + [pltpu.VMEM((1, OFF, QB), f32) for _ in range(NSB)]
              + [pltpu.VMEM((16, QB), f32), pltpu.VMEM((64, QB), u32),
                 pltpu.VMEM((F,), bf16), pltpu.VMEM((D,), bf16)],
            compiler_params=pltpu.CompilerParams(dimension_semantics=("arbitrary",),
                                                 vmem_limit_bytes=127 * 1024 * 1024),
        )(x, A_wqkv, A_wo, B_w1, B_b1, B_w2, B_b2)
        return out.reshape(1, S, D)
    return fn


_FN = make_kernel()


@jax.jit
def pallas_sequential_preLN__softmax_full_mha__dense_activation_gelu__prompt_kernel(
    A_x: jax.Array,
    A_wqkv: jax.Array,
    A_wo: jax.Array,
    B_x: jax.Array,
    B_w1: jax.Array,
    B_b1: jax.Array,
    B_w2: jax.Array,
    B_b2: jax.Array,
):
    return _FN(A_x, A_wqkv, A_wo, B_x, B_w1, B_b1, B_w2, B_b2)
```
